```python
import os as _os
_os.environ.setdefault("JAX_PLATFORMS", "cpu")
import jax
import jax.numpy as jnp

def _softmax(x, axis=-1):
    return jax.nn.softmax(x, axis=axis)
def _gelu(x):
    return jax.nn.gelu(x, approximate=True)
def _silu(x):
    return jax.nn.silu(x)
def _sigmoid(x):
    return jax.nn.sigmoid(x)
def _layernorm(x, axis=-1, eps=1e-5):
    m = jnp.mean(x, axis=axis, keepdims=True)
    v = jnp.var(x, axis=axis, keepdims=True)
    return (x - m) / jnp.sqrt(v + eps)
def _scatter_add(tgt, idx, src, axis=0):
    return tgt.at[idx].add(src)
def _segment_sum(src, seg, n):
    return jax.ops.segment_sum(src, seg, n)
class _Rng:
    def __init__(self, key):
        self._k = key
    def _next(self):
        self._k, sub = jax.random.split(self._k)
        return sub
    def normal(self, shape):
        return jax.random.normal(self._next(), shape, dtype=jnp.bfloat16)
    def randint(self, lo, hi, shape):
        return jax.random.randint(self._next(), shape, lo, hi, dtype=jnp.int32)
    def uniform(self, shape, lo=0.0, hi=1.0):
        return jax.random.uniform(self._next(), shape, jnp.bfloat16, lo, hi)
    def permutation(self, n):
        return jax.random.permutation(self._next(), n)


kernel_name = 'standalone__dense_activation_gelu__prompt'

def setup_inputs():
    _rng = _Rng(jax.random.key(int.from_bytes(__import__("os").urandom(4), "little")))
    _w = (lambda a: (lambda t: t.astype(jnp.bfloat16) if jnp.issubdtype(t.dtype, jnp.floating) else t)(jnp.asarray(a)))
    B, S, D, F = 1, 2048, 640, 1728
    return {
        "x": _w((lambda *s: _rng.normal(s) * 0.05)(B, S, D)),
        "w1": _w((lambda *s: _rng.normal(s) * 0.05)(D, F) * (D ** -0.5)),
        "b1": _w((lambda *s: _rng.normal(s) * 0.05)(F) * 0.01),
        "w2": _w((lambda *s: _rng.normal(s) * 0.05)(F, D) * (F ** -0.5)),
        "b2": _w((lambda *s: _rng.normal(s) * 0.05)(D) * 0.01),
    }

def reference(x, w1, b1, w2, b2):
    h = jnp.einsum("bsd,df->bsf", x, w1) + b1
    h = _gelu(h)
    return jnp.einsum("bsf,fd->bsd", h, w2) + b2
```

```python
import numpy as np

import jax
import jax.numpy as jnp
import jax.experimental.pallas as pl
import jax.experimental.pallas.tpu as pltpu

_NT = (((1,), (1,)), ((), ()))
_C1 = float(np.sqrt(2.0 / np.pi))
_C2 = _C1 * 0.044715

_R = 1280
_STEP_A = (512, 864)
_KS = (128, 256, 256)
_REST = (512, 128, 128)
_REST_FSPLIT = (1, 2, 2)
_LAST_DSPLIT = (384, 256)


def _gelu_x2(h):
    u = h * (h * h * _C2 + _C1)
    return h * jnp.tanh(u) + h


def _ffn_kernel(x_hbm, w1_hbm, b1_hbm, w2_hbm, b2_hbm, o_hbm,
                xb, w1b, b1b, w2b, b2b, ob, w2t, b1cb, sems, osems):
    S, D = x_hbm.shape
    F = w1_hbm.shape[0]
    R, (Ra, Fa), ks = _R, _STEP_A, _KS
    koff = [sum(ks[:i]) for i in range(len(ks))]
    n_in = [0]

    def in_copy(src, dst):
        c = pltpu.make_async_copy(src, dst, sems.at[n_in[0]])
        n_in[0] += 1
        return c

    def x_copy(r0, r1, k0, k1):
        idx = (pl.ds(r0, r1 - r0), pl.ds(k0, k1 - k0))
        return in_copy(x_hbm.at[idx], xb.at[idx])

    def w1_copy(f0, f1, k0, k1):
        idx = (pl.ds(f0, f1 - f0), pl.ds(k0, k1 - k0))
        return in_copy(w1_hbm.at[idx], w1b.at[idx])

    groups = [
        [in_copy(b1_hbm, b1b), in_copy(b2_hbm, b2b)],
        [x_copy(0, Ra, 0, ks[0]), w1_copy(0, Fa, 0, ks[0])],
        [w1_copy(Fa, F, 0, ks[0]), x_copy(Ra, R, 0, ks[0])],
    ]
    for k in range(1, len(ks)):
        k0, k1 = koff[k], koff[k] + ks[k]
        groups.append([w1_copy(0, F, k0, k1), x_copy(0, R, k0, k1)])
    groups[-1] += [
        in_copy(w2_hbm, w2b),
        in_copy(x_hbm.at[pl.ds(R, S - R)], xb.at[pl.ds(R, S - R)]),
    ]
    for g in groups:
        for c in g:
            c.start()
    pending = iter(groups)

    def wait_next():
        for c in next(pending):
            c.wait()

    def mm1(r0, r1, f0, f1, k0, k1):
        return jax.lax.dot_general(
            w1b[pl.ds(f0, f1 - f0), pl.ds(k0, k1 - k0)],
            xb[pl.ds(r0, r1 - r0), pl.ds(k0, k1 - k0)],
            _NT, preferred_element_type=jnp.float32)

    def bias1(f0, f1, n):
        return jnp.concatenate([b1cb[pl.ds(f0, f1 - f0), :]] * (n // 128), axis=1)

    out_copies = []

    def out_copy(o, s, d0, dn):
        idx = (pl.ds(o, s), pl.ds(d0, dn))
        c = pltpu.make_async_copy(ob.at[idx], o_hbm.at[idx],
                                  osems.at[len(out_copies)])
        c.start()
        out_copies.append(c)

    def finish(o, s, hT, dma_dsplit=None):
        gT = _gelu_x2(hT).astype(jnp.bfloat16)
        if dma_dsplit is not None:
            dsplit = dma_dsplit
        elif (s // 128 * pl.cdiv(F, 128)) % 4 == 0:
            dsplit = (D,)
        else:
            dsplit = (D // 2, D // 2)
        d0 = 0
        for dn in dsplit:
            oT = jnp.dot(w2t[pl.ds(d0, dn), :], gT,
                         preferred_element_type=jnp.float32)
            b2 = b2b[pl.ds(d0, dn)].astype(jnp.float32)[None, :]
            ob[pl.ds(o, s), pl.ds(d0, dn)] = (oT.T * 0.5 + b2).astype(ob.dtype)
            if dma_dsplit is not None:
                out_copy(o, s, d0, dn)
            d0 += dn
        if dma_dsplit is None:
            out_copy(o, s, 0, D)

    wait_next()
    b1 = b1b[...].astype(jnp.float32)[None, :]
    b1cb[...] = jnp.broadcast_to(b1, (128, F)).T

    K0 = ks[0]
    wait_next()
    h_aa = mm1(0, Ra, 0, Fa, 0, K0) + bias1(0, Fa, Ra)
    wait_next()
    h_ab = mm1(0, Ra, Fa, F, 0, K0) + bias1(Fa, F, Ra)
    h_ba = mm1(Ra, R, 0, Fa, 0, K0) + bias1(0, Fa, R - Ra)
    h_bb = mm1(Ra, R, Fa, F, 0, K0) + bias1(Fa, F, R - Ra)
    h = jnp.concatenate([jnp.concatenate([h_aa, h_ba], axis=1),
                         jnp.concatenate([h_ab, h_bb], axis=1)], axis=0)
    for k in range(1, len(ks)):
        wait_next()
        if k == len(ks) - 1:
            w2t[...] = w2b[...].T
        h = h + mm1(0, R, 0, F, koff[k], koff[k] + ks[k])
    finish(0, R, h)

    o = R
    for i, (s, n) in enumerate(zip(_REST, _REST_FSPLIT)):
        fq = [F // n * j for j in range(n + 1)]
        hT = jnp.concatenate(
            [mm1(o, o + s, fq[j], fq[j + 1], 0, D) + bias1(fq[j], fq[j + 1], s)
             for j in range(n)], axis=0)
        finish(o, s, hT, _LAST_DSPLIT if i == len(_REST) - 1 else None)
        o += s

    for c in out_copies:
        c.wait()


@jax.jit
def pallas_standalone__dense_activation_gelu__prompt_kernel(
    x: jax.Array,
    w1: jax.Array,
    b1: jax.Array,
    w2: jax.Array,
    b2: jax.Array,
):
    B, S0, D = x.shape
    F = w1.shape[1]
    S = B * S0
    assert S == _R + sum(_REST) and D == sum(_KS) and D == sum(_LAST_DSPLIT)

    n_in = 2 + 2 * (len(_KS) + 1) + 2
    n_out = len(_REST) + len(_LAST_DSPLIT)
    hbm = pl.BlockSpec(memory_space=pltpu.HBM)
    out = pl.pallas_call(
        _ffn_kernel,
        in_specs=[hbm] * 5,
        out_specs=hbm,
        out_shape=jax.ShapeDtypeStruct((S, D), x.dtype),
        scratch_shapes=[
            pltpu.VMEM((S, D), x.dtype),
            pltpu.VMEM((F, D), w1.dtype),
            pltpu.VMEM((F,), b1.dtype),
            pltpu.VMEM((F, D), w2.dtype),
            pltpu.VMEM((D,), b2.dtype),
            pltpu.VMEM((S, D), x.dtype),
            pltpu.VMEM((D, F), w2.dtype),
            pltpu.VMEM((F, 128), jnp.float32),
            pltpu.SemaphoreType.DMA((n_in,)),
            pltpu.SemaphoreType.DMA((n_out,)),
        ],
        compiler_params=pltpu.CompilerParams(
            vmem_limit_bytes=100 * 1024 * 1024,
            disable_semaphore_checks=True,
        ),
    )(x.reshape(S, D), w1.T, b1, w2, b2)
    return out.reshape(B, S0, D)
```

```python
import numpy as np

import jax
import jax.numpy as jnp
import jax.experimental.pallas as pl
import jax.experimental.pallas.tpu as pltpu

_NT = (((1,), (1,)), ((), ()))
_C1 = float(np.sqrt(2.0 / np.pi))
_C2 = _C1 * 0.044715

_R = 1280
_STEP_A = (512, 864)
_KS = (128, 256, 256)
_MID = (384, 256)
_LAST = 128
_LAST_DSPLIT = (256, 256, 128)


def _gelu_x2(h):
    u = h * (h * h * _C2 + _C1)
    return h * jnp.tanh(u) + h


def _ffn_kernel(x_hbm, w1_hbm, b1_hbm, w2_hbm, b2_hbm, o_hbm,
                xb, w1b, b1b, w2b, b2b, ob, w2t, b1cb, in_sems, out_sem):
    S, D = x_hbm.shape
    F = w1_hbm.shape[0]
    R, (Ra, Fa), ks = _R, _STEP_A, _KS
    K0 = ks[0]
    koff = [sum(ks[:i]) for i in range(len(ks))]

    groups = []

    def add_group(*pairs):
        sem = in_sems.at[len(groups)]
        groups.append([pltpu.make_async_copy(s, d, sem) for s, d in pairs])

    def x_piece(r0, r1, k0, k1):
        idx = (pl.ds(r0, r1 - r0), pl.ds(k0, k1 - k0))
        return x_hbm.at[idx], xb.at[idx]

    def w1_piece(f0, f1, k0, k1):
        idx = (pl.ds(f0, f1 - f0), pl.ds(k0, k1 - k0))
        return w1_hbm.at[idx], w1b.at[idx]

    add_group((b1_hbm, b1b), (b2_hbm, b2b))
    add_group(x_piece(0, Ra, 0, K0), w1_piece(0, Fa, 0, K0))
    add_group(w1_piece(Fa, F, 0, K0), x_piece(Ra, R, 0, K0))
    for k in range(1, len(ks)):
        k0, k1 = koff[k], koff[k] + ks[k]
        pairs = [w1_piece(0, F, k0, k1), x_piece(0, R, k0, k1)]
        if k == len(ks) - 1:
            pairs += [(w2_hbm, w2b), x_piece(R, S, 0, D)]
        add_group(*pairs)
    for group in groups:
        for c in group:
            c.start()
    pending = iter(groups)

    def wait_next_group():
        for c in next(pending):
            c.wait()

    def mm1(r0, r1, f0, f1, k0, k1):
        return jax.lax.dot_general(
            w1b[pl.ds(f0, f1 - f0), pl.ds(k0, k1 - k0)],
            xb[pl.ds(r0, r1 - r0), pl.ds(k0, k1 - k0)],
            _NT, preferred_element_type=jnp.float32)

    def bias1(f0, f1, n):
        return jnp.concatenate([b1cb[pl.ds(f0, f1 - f0), :]] * (n // 128), axis=1)

    def bias2(d0, dn):
        return b2b[pl.ds(d0, dn)].astype(jnp.float32)[None, :]

    out_copies = []

    def write_back(o, s, d0, dn):
        idx = (pl.ds(o, s), pl.ds(d0, dn))
        c = pltpu.make_async_copy(ob.at[idx], o_hbm.at[idx], out_sem.at[0])
        c.start()
        out_copies.append(c)

    def finish_transposed(o, s, hT):
        gT = _gelu_x2(hT).astype(jnp.bfloat16)
        n_pass = s // 128 * pl.cdiv(F, 128)
        dsplit = (D,) if n_pass % 4 == 0 else (D // 2, D // 2)
        d0 = 0
        for dn in dsplit:
            oT = jnp.dot(w2t[pl.ds(d0, dn), :], gT,
                         preferred_element_type=jnp.float32)
            ob[pl.ds(o, s), pl.ds(d0, dn)] = (
                oT.T * 0.5 + bias2(d0, dn)).astype(ob.dtype)
            d0 += dn
        write_back(o, s, 0, D)

    wait_next_group()
    b1_row = b1b[...].astype(jnp.float32)[None, :]
    b1cb[...] = jnp.broadcast_to(b1_row, (128, F)).T

    wait_next_group()
    h_aa = mm1(0, Ra, 0, Fa, 0, K0) + bias1(0, Fa, Ra)
    wait_next_group()
    h_ab = mm1(0, Ra, Fa, F, 0, K0) + bias1(Fa, F, Ra)
    h_ba = mm1(Ra, R, 0, F // 2, 0, K0) + bias1(0, F // 2, R - Ra)
    h_bb = mm1(Ra, R, F // 2, F, 0, K0) + bias1(F // 2, F, R - Ra)
    h = jnp.concatenate([jnp.concatenate([h_aa, h_ab], axis=0),
                         jnp.concatenate([h_ba, h_bb], axis=0)], axis=1)
    for k in range(1, len(ks)):
        wait_next_group()
        if k == len(ks) - 1:
            w2t[...] = w2b[...].T
        h = h + mm1(0, R, 0, F, koff[k], koff[k] + ks[k])
    finish_transposed(0, R, h)

    o = R
    for s in _MID:
        finish_transposed(o, s, mm1(o, o + s, 0, F, 0, D) + bias1(0, F, s))
        o += s

    h = jax.lax.dot_general(xb[pl.ds(o, _LAST), :], w1b[...], _NT,
                            preferred_element_type=jnp.float32) + b1_row
    g = _gelu_x2(h).astype(jnp.bfloat16)
    d0 = 0
    for dn in _LAST_DSPLIT:
        r = jnp.dot(g, w2b[:, pl.ds(d0, dn)], preferred_element_type=jnp.float32)
        ob[pl.ds(o, _LAST), pl.ds(d0, dn)] = (r * 0.5 + bias2(d0, dn)).astype(ob.dtype)
        write_back(o, _LAST, d0, dn)
        d0 += dn

    for c in out_copies:
        c.wait()


@jax.jit
def pallas_standalone__dense_activation_gelu__prompt_kernel(
    x: jax.Array,
    w1: jax.Array,
    b1: jax.Array,
    w2: jax.Array,
    b2: jax.Array,
):
    B, S0, D = x.shape
    F = w1.shape[1]
    S = B * S0
    assert S == _R + sum(_MID) + _LAST
    assert D == sum(_KS) and D == sum(_LAST_DSPLIT)

    hbm = pl.BlockSpec(memory_space=pltpu.HBM)
    out = pl.pallas_call(
        _ffn_kernel,
        in_specs=[hbm] * 5,
        out_specs=hbm,
        out_shape=jax.ShapeDtypeStruct((S, D), x.dtype),
        scratch_shapes=[
            pltpu.VMEM((S, D), x.dtype),
            pltpu.VMEM((F, D), w1.dtype),
            pltpu.VMEM((F,), b1.dtype),
            pltpu.VMEM((F, D), w2.dtype),
            pltpu.VMEM((D,), b2.dtype),
            pltpu.VMEM((S, D), x.dtype),
            pltpu.VMEM((D, F), w2.dtype),
            pltpu.VMEM((F, 128), jnp.float32),
            pltpu.SemaphoreType.DMA((len(_KS) + 2,)),
            pltpu.SemaphoreType.DMA((1,)),
        ],
        compiler_params=pltpu.CompilerParams(
            vmem_limit_bytes=100 * 1024 * 1024),
    )(x.reshape(S, D), w1.T, b1, w2, b2)
    return out.reshape(B, S0, D)
```
